```python
import os as _os
_os.environ.setdefault("JAX_PLATFORMS", "cpu")
import jax
import jax.numpy as jnp

def _softmax(x, axis=-1):
    return jax.nn.softmax(x, axis=axis)
def _gelu(x):
    return jax.nn.gelu(x, approximate=True)
def _silu(x):
    return jax.nn.silu(x)
def _sigmoid(x):
    return jax.nn.sigmoid(x)
def _layernorm(x, axis=-1, eps=1e-5):
    m = jnp.mean(x, axis=axis, keepdims=True)
    v = jnp.var(x, axis=axis, keepdims=True)
    return (x - m) / jnp.sqrt(v + eps)
def _scatter_add(tgt, idx, src, axis=0):
    return tgt.at[idx].add(src)
def _segment_sum(src, seg, n):
    return jax.ops.segment_sum(src, seg, n)
class _Rng:
    def __init__(self, key):
        self._k = key
    def _next(self):
        self._k, sub = jax.random.split(self._k)
        return sub
    def normal(self, shape):
        return jax.random.normal(self._next(), shape, dtype=jnp.bfloat16)
    def randint(self, lo, hi, shape):
        return jax.random.randint(self._next(), shape, lo, hi, dtype=jnp.int32)
    def uniform(self, shape, lo=0.0, hi=1.0):
        return jax.random.uniform(self._next(), shape, jnp.bfloat16, lo, hi)
    def permutation(self, n):
        return jax.random.permutation(self._next(), n)


kernel_name = 'gated_mix__compressed_kv_cla__ssm_conv_h3__prompt'

def setup_inputs():
    _rng = _Rng(jax.random.key(int.from_bytes(__import__("os").urandom(4), "little")))
    _w = (lambda a: (lambda t: t.astype(jnp.bfloat16) if jnp.issubdtype(t.dtype, jnp.floating) else t)(jnp.asarray(a)))
    def _A_setup():
        B, H, Sq, Sk, D, M = 1, 32, 2048, 2048, 128, 1024
        Dc = 4 * D
        return {
            "x": _w((lambda *s: _rng.normal(s) * 0.05)(B, Sq, M)),
            "c_kv": _w((lambda *s: _rng.normal(s) * 0.8)(B, Sk, Dc)),
            "w_q": _w((lambda *s: _rng.normal(s) * 3.2)(M, H, D) * (M ** -0.5)),
            "w_uk": _w((lambda *s: _rng.normal(s) * 3.2)(Dc, H, D) * (Dc ** -0.5)),
            "w_uv": _w((lambda *s: _rng.normal(s) * 0.8)(Dc, H, D) * (Dc ** -0.5)),
            "w_o": _w((lambda *s: _rng.normal(s) * 0.8)(H, D, M) * ((H * D) ** -0.5)),
        }
    _A_in = _A_setup()

    def _B_setup():
        B, S, D = 1, 2048, 1024
        ks = 4
        return {
            "q": _w((lambda *s: _rng.normal(s) * 0.05)(B, S, D)),
            "k": _w((lambda *s: _rng.normal(s) * 0.8)(B, S, D)),
            "v": _w((lambda *s: _rng.normal(s) * 0.8)(B, S, D)),
            "shift_k": _w((lambda *s: _rng.normal(s) * 0.8)(D, ks) * 0.5),
            "ssm_k": _w((lambda *s: _rng.normal(s) * 0.8)(D, S) * (1.0 / S ** 0.5)),
            "ssm_D": _w((lambda *s: _rng.normal(s) * 0.8)(D)),
        }
    _B_in = _B_setup()

    return {
        "A_x": _A_in["x"],
        "A_c_kv": _A_in["c_kv"],
        "A_w_q": _A_in["w_q"],
        "A_w_uk": _A_in["w_uk"],
        "A_w_uv": _A_in["w_uv"],
        "A_w_o": _A_in["w_o"],
        "B_q": _B_in["q"],
        "B_k": _B_in["k"],
        "B_v": _B_in["v"],
        "B_shift_k": _B_in["shift_k"],
        "B_ssm_k": _B_in["ssm_k"],
        "B_ssm_D": _B_in["ssm_D"],
        "gate_w": _w((lambda *s: _rng.normal(s) * 0.05)(1024) * 16.0),
    }

def reference(A_x, A_c_kv, A_w_q, A_w_uk, A_w_uv, A_w_o, B_q, B_k, B_v, B_shift_k, B_ssm_k, B_ssm_D, gate_w):
    def _A_ref(x, c_kv, w_q, w_uk, w_uv, w_o):
        B, Sq, M = x.shape[0], x.shape[1], x.shape[2]
        Sk = c_kv.shape[1]
        H, D = w_q.shape[1], w_q.shape[2]
        q = jnp.einsum("bqm,mhd->bhqd", x, w_q)
        k = jnp.einsum("bkc,chd->bhkd", c_kv, w_uk)
        v = jnp.einsum("bkc,chd->bhkd", c_kv, w_uv)
        scores = jnp.einsum("bhqd,bhkd->bhqk", q, k) * (D ** -0.5)
        off = Sk - Sq
        qi = jnp.arange(Sq)[:, None]
        kj = jnp.arange(Sk)[None, :]
        cmask = kj <= (qi + off)
        scores = jnp.where(cmask[None, None], scores, -1e9)
        p = _softmax(scores, axis=-1)
        ctx = jnp.einsum("bhqk,bhkd->bhqd", p, v)
        return jnp.einsum("bhqd,hdm->bqm", ctx, w_o)

    def _B_ref(q, k, v, shift_k, ssm_k, ssm_D):
        B, S, D = q.shape
        ks = shift_k.shape[-1]
        k_pad = jnp.pad(k, ((0, 0), (ks - 1, 0), (0, 0)))
        k_shift = jnp.zeros_like(k)
        for t in range(ks):
            k_shift = k_shift + k_pad[:, t:t + S, :] * shift_k[:, ks - 1 - t][None, None, :]
        kv = k_shift * v
        L = 2 * S
        kv_pad = jnp.pad(kv, ((0, 0), (0, S), (0, 0)))
        kf_pad = jnp.pad(ssm_k, ((0, 0), (0, S)))
        kv_f = (lambda x, axes=(-2,-1): jnp.fft.rfft2(x.astype(jnp.float32), axes=axes))(kv_pad[:, None, :, :], axes=(1, 2))
        kf_f = (lambda x, axes=(-2,-1): jnp.fft.rfft2(x.astype(jnp.float32), axes=axes))(kf_pad[:, None, :], axes=(1, 2))
        kf_f = (lambda x, *d: x.transpose(*d))(kf_f, 1, 2, 0)
        y_f = kv_f * kf_f[None, :, :, :]
        y = (lambda x, s, axes=(-2,-1): jnp.fft.irfft2(x, s=s, axes=axes).astype(jnp.bfloat16))(y_f, (1, L), axes=(1, 2))[:, 0, :S, :]
        y = y + kv * ssm_D[None, None, :]
        return q * y

    x = A_x
    g = _sigmoid((x * gate_w).sum(-1, keepdims=True))
    a = _A_ref(x, A_c_kv, A_w_q, A_w_uk, A_w_uv, A_w_o)
    b = _B_ref(x, B_k, B_v, B_shift_k, B_ssm_k, B_ssm_D)
    return g * a + (1 - g) * b
```

```python
import math

import jax
import jax.numpy as jnp
import numpy as np
from jax import lax
from jax.experimental import pallas as pl
from jax.experimental.pallas import tpu as pltpu

S, M, DC, H, D = 2048, 1024, 512, 32, 128
NP = H // 2
T = 128
NB = S // T
CB = 256
NCB = M // CB
f32, bf16, u32 = jnp.float32, jnp.bfloat16, jnp.uint32
NT = (((1,), (1,)), ((), ()))
QSCALE = D ** -0.5 * math.log2(math.e)


def _dft_matrices():
    even = np.arange(0, T, 2).reshape(-1, 8)
    bins = np.concatenate([even, T - 1 - even], 1).reshape(-1)
    ang = np.pi * (bins[:, None] + 0.5) * np.arange(T)[None, :] / T
    fwd = np.concatenate([np.cos(ang), -np.sin(ang)], 0)
    t = np.concatenate([np.arange(0, T, 2), np.arange(1, T, 2)])
    ang = np.pi * (even[None] + 0.5) * t[:, None, None] / T
    inv = np.concatenate([np.cos(ang), -np.sin(ang)], 2).reshape(T, T) / T
    return fwd.astype(bf16), inv.astype(bf16)


def _pack(v):
    return pltpu.bitcast(v.astype(bf16), u32)


def _unpack(w):
    return pltpu.bitcast(w, bf16)


def _dot(a, b):
    return jnp.dot(a, b, preferred_element_type=f32)


def _dot_nt(a, b):
    return lax.dot_general(a, b, NT, preferred_element_type=f32)


def _weave(ev, od, g=16):
    return jnp.concatenate([t[i:i + g] for i in range(0, ev.shape[0], g) for t in (ev, od)], axis=0)


def _unweave(v, g=16):
    rows = range(0, v.shape[0], 2 * g)
    return (jnp.concatenate([v[i:i + g] for i in rows], axis=0),
            jnp.concatenate([v[i + g:i + 2 * g] for i in rows], axis=0))


def _fold(op, xs):
    acc = xs[0]
    for x in xs[1:]:
        acc = op(acc, x)
    return acc


def _plans():
    blk = lambda kind, e, i, n=256: (kind, e, i * n, (i + 1) * n)
    loop = [blk("qk", e, i) for i in (1, 0) for e in (0, 1)]
    loop += [blk("pv", e, i) for i in (1, 0) for e in (0, 1)]
    loop += [blk("qk", 0, 7), blk("q", 0, 0), blk("q", 0, 1), blk("pv", 0, 7),
             blk("qk", 1, 7), blk("q", 0, 7), blk("pv", 1, 7)]
    for i in range(6, 1, -1):
        loop += [blk("qk", 0, i), blk("kv", 0, i + 1), blk("pv", 0, i),
                 blk("qk", 1, i), blk("q", 0, i), blk("pv", 1, i)]
    loop += [blk("kv", 0, i) for i in (2, 1, 0)]
    seq = [(e, i) for pair in zip(range(8), range(15, 7, -1)) for i in pair for e in (0, 1)]
    last = []
    for n, (e, i) in enumerate(seq):
        last.append(blk("qk", e, i, 128))
        if n >= 2:
            last.append(blk("pv", *seq[n - 2], 128))
    last += [blk("pv", e, i, 128) for e, i in seq[-2:]]
    return loop, last


def make(C_ROWS=(0, 256, 768, S), X_ROWS=(0, 768, 1536, S), OM=512, INV_AT=3, T0=1200, T1=21000, GD=-2, GL=0,
         ORD=(1, 3, 0, 4, 6, 2, 5), HLEAD=2, nbc=True):
    def _lhs_terms(a11, a12, a21, a22):
        t = [a11 + a22, a21 + a22, a11, a22, a11 + a12, a21 - a11, a12 - a22]
        return [t[i] for i in ORD]

    def _rhs_terms(b11, b12, b21, b22):
        t = [b11 + b22, b11, b12 - b22, b21 - b11, b22, b11 + b12, b21 + b22]
        return [t[i] for i in ORD]

    def _combine(p):
        m = [p[ORD.index(i)] for i in range(7)]
        return (_weave(m[0] + m[3] - m[4] + m[6], m[1] + m[3]),
                _weave(m[2] + m[4], m[0] - m[1] + m[2] + m[5]))

    def kernel(x_hbm, c_hbm, wq_hbm, wuk_hbm, wuv_hbm, wo_hbm, bk_hbm, bv_hbm, h_hbm,
               sk_hbm, sd_hbm, gw_hbm, fwd_hbm, inv_hbm, o_hbm,
               sk_v, sd_v, gw_v, fwd_v, inv_v, x_v, c_v, xs_v, cs_v, w_v, q_v, k_v, v_v, ctx_v,
               wo_v, bk_v, bv_v, h_v, g_v, row_v, kp_v, ud_v, U_v, H_v, Y_v, y_v, o_v,
               csem, xsem, wsem, bsem, osem, ssem):
        copy = pltpu.make_async_copy

        def weight_copies(j, slot):
            parts = ((wq_hbm, 0, M), (wuk_hbm, M, DC), (wuv_hbm, M + DC, DC))
            return [copy(w.bitcast(u32).at[:, j, :], w_v.at[slot, pl.ds(a, n)], wsem.at[slot, i])
                    for i, (w, a, n) in enumerate(parts)]

        def channels(cb):
            return pl.ds(cb * CB if isinstance(cb, int) else pl.multiple_of(cb * CB, CB), CB)

        def block_copies(cb, slot):
            cs = channels(cb)
            return [copy(wo_hbm.at[:, :, cs], wo_v.at[slot], bsem.at[slot, 0]),
                    copy(bk_hbm.at[:, cs], bk_v.at[slot], bsem.at[slot, 1]),
                    copy(bv_hbm.at[:, cs], bv_v.at[slot], bsem.at[slot, 2]),
                    copy(h_hbm.at[cs, :], h_v.at[slot], bsem.at[slot, 3])]

        def out_copy(cb, slot, part):
            cut = INV_AT * OM
            rs = pl.ds(cut, S - cut) if part else pl.ds(0, cut)
            return copy(o_v.at[slot, rs], o_hbm.at[rs, channels(cb)], osem.at[slot, part])

        def row_copies(src, dst, sem, cuts):
            return [copy(src.at[pl.ds(a, b - a)], dst.at[pl.ds(a, b - a)], sem.at[i])
                    for i, (a, b) in enumerate(zip(cuts, cuts[1:]))]

        def weight_terms(slot, a, n):
            halves = []
            for r in (a, a + n // 2):
                w = w_v[slot, pl.ds(r, n // 2), :]
                halves += [pltpu.bitcast(w << 16, f32), pltpu.bitcast(w & np.uint32(0xFFFF0000), f32)]
            return _rhs_terms(*halves)

        def q_weights(slot):
            return [t.astype(bf16) for t in weight_terms(slot, 0, M)]

        def kv_weights(slot):
            return [jnp.concatenate(t, axis=1).astype(bf16)
                    for t in zip(weight_terms(slot, M, DC), weight_terms(slot, M + DC, DC))]

        def project_q(lhs, wts, a, b):
            for e, t in enumerate(_combine([_dot(_unpack(l), w) for l, w in zip(lhs, wts)])):
                q_v[e, a:b] = (t * QSCALE).astype(bf16)

        def project_kv(lhs, wts, a, b):
            for e, t in enumerate(_combine([_dot(_unpack(l), w) for l, w in zip(lhs, wts)])):
                k_v[e, a:b] = t[:, :D].astype(bf16)
                v_v[e, a:b] = t[:, D:].astype(bf16)

        def scores(qb, e, a, b):
            tri = (lax.broadcasted_iota(jnp.int32, (128, 128), 1)
                   <= lax.broadcasted_iota(jnp.int32, (128, 128), 0))
            full = _dot_nt(qb, k_v[e, 0:a + 128])
            stairs = {t: _dot_nt(q_v[e, t:b], k_v[e, t:t + 128]) for t in range(a + 128, b, 128)}
            rows = []
            for r in range(a, b, 128):
                tiles = [full[r - a:r - a + 128, t:t + 128] for t in range(0, a + 128, 128)]
                tiles += [s[r - t:r - t + 128] for t, s in stairs.items() if t <= r]
                tiles[-1] = jnp.where(tri, tiles[-1], -1e30)
                rows.append(tiles)
            return rows

        def attend(rows, e, a, b):
            ps, sums = [], []
            for tiles in rows:
                top = jnp.max(_fold(jnp.maximum, tiles), axis=1, keepdims=True)
                ps.append([jnp.exp2(t - top) for t in tiles])
                sums.append(jnp.sum(_fold(jnp.add, ps[-1]), axis=1, keepdims=True))
            n0 = a // 128 + 1
            p = jnp.concatenate([jnp.concatenate(t[:n0], axis=1) for t in ps], axis=0)
            acc = _dot(p.astype(bf16), v_v[e, 0:a + 128])
            accs = [acc[i * 128:(i + 1) * 128] for i in range(len(ps))]
            for s in range(1, len(ps)):
                p = jnp.concatenate([t[n0 + s - 1] for t in ps[s:]], axis=0)
                acc = _dot(p.astype(bf16), v_v[e, a + s * 128:a + (s + 1) * 128])
                for i in range(s, len(ps)):
                    accs[i] = accs[i] + acc[(i - s) * 128:(i - s + 1) * 128]
            out = []
            for acc, l in zip(accs, sums):
                r = pl.reciprocal(l, approx=True)
                out.append(acc * (r * (2.0 - l * r)))
            return out

        def head_pair(plan, j, slot):
            zero = (j >> 8).astype(u32)
            own = pl.ds(pl.multiple_of(j * 128, 128), 128)
            gate = jax.nn.sigmoid(jnp.sum(x_v[own].astype(f32) * row_v[5:6], axis=1, keepdims=True))
            gate = jnp.broadcast_to(gate, (128, 128))
            g_v[own] = gate
            bits = pltpu.bitcast(gate, u32)
            waiting = [(GD if slot is not None else GL,
                        _fold(jnp.bitwise_or, [bits[i:i + 32] for i in range(0, 128, 32)]) & zero)]
            if slot is not None:
                wq, wkv = q_weights(slot), kv_weights(slot)
            step, pending, ctx = 0, {}, {}

            def paced(ref, a, b):
                lhs = [ref[i, a // 4:b // 4] for i in range(7)]
                for i in (2, 4, 6):
                    if waiting and waiting[0][0] + 1 < step:
                        w, word = lhs[i], waiting.pop(0)[1]
                        ev, od = _unweave(w[:, :128], 8)
                        lhs[i] = jnp.concatenate([_weave(ev | word, od, 8), w[:, 128:]], axis=1)
                return lhs

            for kind, e, a, b in plan:
                if kind == "q":
                    step += 1
                    project_q(paced(xs_v, a, b), wq, a, b)
                elif kind == "kv":
                    step += 1
                    project_kv(paced(cs_v, a, b), wkv, a, b)
                elif kind == "qk":
                    qb = q_v[e, a:b]
                    if slot is None:
                        step += 1
                        if waiting and waiting[0][0] + 3 < step:
                            w = pltpu.bitcast(qb, u32)
                            qb = _unpack(jnp.concatenate([w[:32] | waiting.pop(0)[1], w[32:]], axis=0))
                    pending[e, a] = scores(qb, e, a, b)
                else:
                    for r, c in zip(range(a, b, 128), attend(pending.pop((e, a)), e, a, b)):
                        ctx[e, r] = c
                        if (1 - e, r) in ctx:
                            (a11, a21), (a12, a22) = _unweave(ctx[0, r]), _unweave(ctx[1, r])
                            terms = [_pack(t) for t in _lhs_terms(a11, a12, a21, a22)]
                            for i, t in enumerate(terms):
                                ctx_v[i, r // 4:(r + 128) // 4, own] = t
                            waiting.append((step, _fold(jnp.bitwise_or, terms) & zero))

        def input_terms(src, dst, a, b):
            ev, od = _unweave(src[a:b].astype(f32))
            n = ev.shape[1] // 2
            terms = [_pack(t) for t in _lhs_terms(ev[:, :n], ev[:, n:], od[:, :n], od[:, n:])]
            for i, t in enumerate(terms):
                dst[i, a // 4:b // 4] = t
            return terms

        c_in = row_copies(c_hbm, c_v, csem, C_ROWS)
        x_in = row_copies(x_hbm, x_v, xsem, X_ROWS)
        w_in = weight_copies(0, 0)
        small = [copy(a, b, ssem.at[i]) for i, (a, b) in enumerate(
            ((sk_hbm, sk_v), (sd_hbm, sd_v), (gw_hbm, gw_v), (fwd_hbm, fwd_v), (inv_hbm, inv_v)))]
        for cp in (c_in[0], w_in[1], w_in[2], c_in[1]):
            cp.start()
        w_in[1].wait()
        w_in[2].wait()
        for i, then in enumerate(([c_in[2]], [w_in[0], x_in[0], x_in[1]], x_in[2:])):
            c_in[i].wait()
            for cp in then:
                cp.start()
            if i == 0:
                wkv = kv_weights(0)
            for a in range(C_ROWS[i], C_ROWS[i + 1], 256):
                project_kv(input_terms(c_v, cs_v, a, a + 256), wkv, a, a + 256)
        w_in[0].wait()
        for i, cp in enumerate(x_in):
            cp.wait()
            if i == 0:
                wq = q_weights(0)
            if i == 1:
                for cp in small + weight_copies(1, 1):
                    cp.start()
            for a in range(X_ROWS[i], X_ROWS[i + 1], 256):
                project_q(input_terms(x_v, xs_v, a, a + 256), wq, a, a + 256)
        for cp in small:
            cp.wait()
        row_v[0:4] = sk_v[...].astype(f32)
        row_v[4:5] = sd_v[...].astype(f32).reshape(1, M)
        row_v[5:6] = gw_v[...].astype(f32).reshape(1, M)

        loop_plan, last_plan = _plans()

        def pair_step(j, _):
            slot = (j + 1) % 2
            for cp in weight_copies(j + 1, slot):
                cp.wait()

            @pl.when(j + 2 < NP)
            def _():
                for cp in weight_copies(j + 2, 1 - slot):
                    cp.start()

            head_pair(loop_plan, j, slot)
            return j + 1

        j_last = lax.fori_loop(0, NP - 1, pair_step, 0)
        for cp in block_copies(0, 0):
            cp.start()
        head_pair(last_plan, j_last, None)

        kp_v[0:8] = jnp.zeros((8, CB), f32)

        def spectra(slot, cs):
            fwd = fwd_v[...]
            taps = row_v[0:5, cs]
            prev = None
            for n in range(NB + HLEAD):
                if n < NB:
                    cur = _dot_nt(fwd, h_v[slot, :, n * T:(n + 1) * T])
                    if prev is None:
                        H_v[n] = cur
                    else:
                        (r0, r1), (i0, i1) = _unweave(cur[:T], 8), _unweave(cur[T:], 8)
                        (pr0, pr1), (pi0, pi1) = _unweave(prev[:T], 8), _unweave(prev[T:], 8)
                        H_v[n, :T] = _weave(r0 - pi0, r1 + pi1, 8)
                        H_v[n, T:] = _weave(i0 + pr0, i1 - pr1, 8)
                    prev = cur
                if n >= HLEAD:
                    a = n - HLEAD
                    r = a * T
                    kp_v[8 + r:8 + r + T] = bk_v[slot, r:r + T].astype(f32)
                    ks = _fold(jnp.add, [kp_v[pl.ds(8 + r - t, T)] * taps[t:t + 1] for t in range(4)])
                    u = ks * bv_v[slot, r:r + T].astype(f32)
                    ud_v[r:r + T] = u * taps[4:5]
                    U_v[a] = _dot(fwd, u.astype(bf16))

        def block_convolution(zero):
            words, done, total = {}, 0, (CB // 128) * (T // 16) * NB * (NB + 1) // 2

            def pace(w):
                tick = int(T0 + (T1 - T0) * done / total) // 16
                words[tick] = words[tick] | (w & zero) if tick in words else w & zero

            for c in range(0, CB, 128):
                ln = slice(c, c + 128)
                for f in range(0, T, 16):
                    re, im = slice(f, f + 16), slice(T + f, T + f + 16)
                    for a0 in range(0, NB, 2):
                        yr, yi, hs = [None, None], [None, None], {}
                        for s in range(a0 + 2):
                            ur, ui = U_v[s, re, ln], U_v[s, im, ln]
                            for o in range(2):
                                d = a0 + o - s
                                if d < 0:
                                    continue
                                if d not in hs:
                                    hs[d] = H_v[d, re, ln], H_v[d, im, ln]
                                hr, hi = hs[d]
                                pr, pi = hr * ur - hi * ui, hr * ui + hi * ur
                                yr[o] = pr if s == 0 else yr[o] + pr
                                yi[o] = pi if s == 0 else yi[o] + pi
                                done += 1
                            if s % 2 == 1 and s <= a0:
                                w = _fold(jnp.bitwise_or, [pltpu.bitcast(t, u32) for t in yr + yi])
                                pace(w[:8] | w[8:])
                        outs = []
                        for o in range(2):
                            r0, r1, i0, i1 = yr[o][:8], yr[o][8:], yi[o][:8], yi[o][8:]
                            for off, parts in ((0, (r0 + r1, i0 - i1)), (T, (r0 - r1, i0 + i1))):
                                outs.append(_pack(jnp.concatenate(parts, axis=0)))
                                Y_v[a0 + o, (off + f) // 2:(off + f) // 2 + 8, ln] = outs[-1]
                        pace(_fold(jnp.bitwise_or, outs))
            return words

        def channel_step(cb, _):
            slot = cb % 2
            cs = channels(cb)
            for cp in block_copies(cb, slot):
                cp.wait()
            spectra(slot, cs)

            @pl.when(cb + 1 < NCB)
            def _():
                for cp in block_copies(cb + 1, 1 - slot):
                    cp.start()

            @pl.when(cb >= 2)
            def _():
                out_copy(cb - 2, slot, 0).wait()
                out_copy(cb - 2, slot, 1).wait()

            inv = inv_v[...]
            words = block_convolution((cb >> 8).astype(u32))
            wo = [jnp.concatenate([wo_v[slot, 2 * p + e, :, n:n + 128] for p in range(NP)], axis=0).astype(f32)
                  for e in range(2) for n in (0, 128)]
            wo = [t.astype(bf16) for t in _rhs_terms(*wo)]
            att, ssm, tick = {}, {}, 0

            def mix(lo, hi):
                for r in range(lo, hi, T):
                    g = g_v[r:r + T]
                    g = jnp.concatenate([g, g], axis=1)
                    o_v[slot, r:r + T] = (ssm[r] + g * (att[r] - ssm[r])).astype(bf16)

            for n, lo in enumerate(range(0, S, OM)):
                if n == INV_AT:
                    for a in range(NB):
                        r = a * T
                        for par in range(2):
                            hf = slice(par * T // 2, (par + 1) * T // 2)
                            y = _dot(inv[hf], _unpack(Y_v[a, hf]))
                            for c in range(CB // 128):
                                y_v[c, pl.ds(r + par, T // 2, stride=2), :] = y[:, c * 128:(c + 1) * 128]
                        y = jnp.concatenate([y_v[c, r:r + T] for c in range(CB // 128)], axis=1)
                        ssm[r] = x_v[r:r + T, cs].astype(f32) * (y + ud_v[r:r + T])
                    mix(0, lo)
                    out_copy(cb, slot, 0).start()
                prods = []
                for i in range(7):
                    cols = []
                    for k in range(0, NP * D, 512):
                        rows = []
                        for r in range(lo // 4, (lo + OM) // 4, 8):
                            w = ctx_v[i, r:r + 8, k:k + 128]
                            rows.append(w | words[tick] if tick in words else w)
                            tick += 1
                        cols += [jnp.concatenate(rows, axis=0),
                                 ctx_v[i, lo // 4:(lo + OM) // 4, k + 128:k + 512]]
                    prods.append(_dot(_unpack(jnp.concatenate(cols, axis=1)), wo[i]))
                o = jnp.concatenate(_combine(prods), axis=1)
                for r in range(lo, lo + OM, T):
                    att[r] = o[r - lo:r - lo + T]
                if n >= INV_AT:
                    mix(lo, lo + OM)
            out_copy(cb, slot, 1).start()

        lax.fori_loop(0, NCB, channel_step, None)
        for cb in (NCB - 2, NCB - 1):
            out_copy(cb, cb % 2, 0).wait()
            out_copy(cb, cb % 2, 1).wait()

    def call(A_x, A_c_kv, A_w_q, A_w_uk, A_w_uv, A_w_o, B_q, B_k, B_v, B_shift_k, B_ssm_k, B_ssm_D, gate_w):
        del B_q
        vmem, sems = pltpu.VMEM, pltpu.SemaphoreType.DMA
        hbm = pl.BlockSpec(memory_space=pl.ANY)
        out = pl.pallas_call(
            kernel,
            out_shape=jax.ShapeDtypeStruct((S, M), bf16),
            in_specs=[hbm] * 14,
            out_specs=hbm,
            scratch_shapes=[
                vmem((4, M), bf16), vmem((M,), bf16), vmem((M,), bf16),
                vmem((2 * T, T), bf16), vmem((T, T), bf16),
                vmem((S, M), bf16), vmem((S, DC), bf16),
                vmem((7, S // 4, M // 2), u32), vmem((7, S // 4, DC // 2), u32),
                vmem((2, M + 2 * DC, D), u32),
                vmem((2, S, D), bf16), vmem((2, S, D), bf16), vmem((2, S, D), bf16),
                vmem((7, S // 4, NP * D), u32),
                vmem((2, H, D, CB), bf16), vmem((2, S, CB), bf16), vmem((2, S, CB), bf16),
                vmem((2, CB, S), bf16),
                vmem((S, 128), f32), vmem((8, M), f32), vmem((S + 8, CB), f32), vmem((S, CB), f32),
                vmem((NB, 2 * T, CB), f32), vmem((NB, 2 * T, CB), f32), vmem((NB, T, CB), u32),
                vmem((CB // 128, S + 8, 128), f32), vmem((2, S, CB), bf16),
                sems((len(C_ROWS) - 1,)), sems((len(X_ROWS) - 1,)), sems((2, 3)), sems((2, 4)),
                sems((2, 2)), sems((5,)),
            ],
            compiler_params=pltpu.CompilerParams(vmem_limit_bytes=120 * 2**20, disable_bounds_checks=nbc),
        )(A_x.reshape(S, M), A_c_kv.reshape(S, DC), A_w_q, A_w_uk, A_w_uv, A_w_o,
          B_k.reshape(S, M), B_v.reshape(S, M), B_ssm_k, B_shift_k.T, B_ssm_D, gate_w,
          *_dft_matrices())
        return out.reshape(1, S, M)
    return call


@jax.jit
def pallas_gated_mix__compressed_kv_cla__ssm_conv_h3__prompt_kernel(
    A_x, A_c_kv, A_w_q, A_w_uk, A_w_uv, A_w_o, B_q, B_k, B_v, B_shift_k, B_ssm_k, B_ssm_D, gate_w,
):
    return make()(A_x, A_c_kv, A_w_q, A_w_uk, A_w_uv, A_w_o, B_q, B_k, B_v, B_shift_k, B_ssm_k, B_ssm_D, gate_w)
```

```python
import math

import jax
import jax.numpy as jnp
import numpy as np
from jax import lax
from jax.experimental import pallas as pl
from jax.experimental.pallas import tpu as pltpu

S, M, DC, H, D = 2048, 1024, 512, 32, 128
NP = H // 2
T = 128
NB = S // T
CB = 256
NCB = M // CB
C_ROWS = (0, 256, 1024, S)
X_ROWS = (0, 512, 1024, 1536, S)
OM = 512
INV_AT = 3
H_LEAD = 2
PACE_FROM, PACE_TO = 2500, 21000
f32, bf16, u32 = jnp.float32, jnp.bfloat16, jnp.uint32
NT = (((1,), (1,)), ((), ()))
QSCALE = D ** -0.5 * math.log2(math.e)


def _dft_matrices():
    even = np.arange(0, T, 2).reshape(-1, 8)
    bins = np.concatenate([even, T - 1 - even], 1).reshape(-1)
    ang = np.pi * (bins[:, None] + 0.5) * np.arange(T)[None, :] / T
    fwd = np.concatenate([np.cos(ang), -np.sin(ang)], 0)
    t = np.concatenate([np.arange(0, T, 2), np.arange(1, T, 2)])
    ang = np.pi * (even[None] + 0.5) * t[:, None, None] / T
    inv = np.concatenate([np.cos(ang), -np.sin(ang)], 2).reshape(T, T) / T
    return fwd.astype(bf16), inv.astype(bf16)


def _pack(v):
    return pltpu.bitcast(v.astype(bf16), u32)


def _unpack(w):
    return pltpu.bitcast(w, bf16)


def _dot(a, b):
    return jnp.dot(a, b, preferred_element_type=f32)


def _dot_nt(a, b):
    return lax.dot_general(a, b, NT, preferred_element_type=f32)


def _weave(ev, od, g=16):
    return jnp.concatenate([t[i:i + g] for i in range(0, ev.shape[0], g) for t in (ev, od)], axis=0)


def _unweave(v, g=16):
    rows = range(0, v.shape[0], 2 * g)
    return (jnp.concatenate([v[i:i + g] for i in rows], axis=0),
            jnp.concatenate([v[i + g:i + 2 * g] for i in rows], axis=0))


def _fold(op, xs):
    acc = xs[0]
    for x in xs[1:]:
        acc = op(acc, x)
    return acc


def _plans():
    blk = lambda kind, e, i, n=256: (kind, e, i * n, (i + 1) * n)
    loop = [blk("qk", 0, 1), blk("qk", 1, 1), blk("pv", 0, 1), blk("pv", 1, 1),
            blk("qk", 0, 0), blk("qk", 1, 0), blk("q", 0, 1), blk("pv", 0, 0), blk("pv", 1, 0),
            blk("qk", 0, 7), blk("q", 0, 0), blk("pv", 0, 7),
            blk("qk", 1, 7), blk("q", 0, 7), blk("pv", 1, 7)]
    for i in range(6, 1, -1):
        loop += [blk("qk", 0, i), blk("kv", 0, i + 1), blk("pv", 0, i),
                 blk("qk", 1, i), blk("q", 0, i), blk("pv", 1, i)]
    loop += [blk("kv", 0, i) for i in (2, 1, 0)]
    seq = [(e, i) for pair in zip(range(8), range(15, 7, -1)) for i in pair for e in (0, 1)]
    last = []
    for n, (e, i) in enumerate(seq):
        last.append(blk("qk", e, i, 128))
        if n >= 2:
            last.append(blk("pv", *seq[n - 2], 128))
    last += [blk("pv", e, i, 128) for e, i in seq[-2:]]
    return loop, last


def _lhs_terms(a11, a12, a21, a22):
    return [a21 + a22, a22, a11 + a22, a11 + a12, a12 - a22, a11, a21 - a11]


def _rhs_terms(b11, b12, b21, b22):
    return [b11, b21 - b11, b11 + b22, b22, b21 + b22, b12 - b22, b11 + b12]


def _combine(products):
    m2, m4, m1, m5, m7, m3, m6 = products
    return _weave(m1 + m4 - m5 + m7, m2 + m4), _weave(m3 + m5, m1 - m2 + m3 + m6)


def _kernel(x_hbm, c_hbm, wq_hbm, wuk_hbm, wuv_hbm, wo_hbm, bk_hbm, bv_hbm, h_hbm,
            sk_hbm, sd_hbm, gw_hbm, fwd_hbm, inv_hbm, o_hbm,
            sk_v, sd_v, gw_v, fwd_v, inv_v, x_v, c_v, xs_v, cs_v, w_v, q_v, k_v, v_v, ctx_v,
            wo_v, bk_v, bv_v, h_v, g_v, row_v, kp_v, ud_v, U_v, H_v, Y_v, y_v, o_v,
            csem, xsem, wsem, bsem, osem, ssem):
    copy = pltpu.make_async_copy

    def weight_copies(j, slot):
        parts = ((wq_hbm, 0, M), (wuk_hbm, M, DC), (wuv_hbm, M + DC, DC))
        return [copy(w.bitcast(u32).at[:, j, :], w_v.at[slot, pl.ds(a, n)], wsem.at[slot, i])
                for i, (w, a, n) in enumerate(parts)]

    def channels(cb):
        return pl.ds(cb * CB if isinstance(cb, int) else pl.multiple_of(cb * CB, CB), CB)

    def block_copies(cb, slot):
        cs = channels(cb)
        return [copy(wo_hbm.at[:, :, cs], wo_v.at[slot], bsem.at[slot, 0]),
                copy(bk_hbm.at[:, cs], bk_v.at[slot], bsem.at[slot, 1]),
                copy(bv_hbm.at[:, cs], bv_v.at[slot], bsem.at[slot, 2]),
                copy(h_hbm.at[cs, :], h_v.at[slot], bsem.at[slot, 3])]

    def out_copy(cb, slot, part):
        cut = INV_AT * OM
        rs = pl.ds(cut, S - cut) if part else pl.ds(0, cut)
        return copy(o_v.at[slot, rs], o_hbm.at[rs, channels(cb)], osem.at[slot, part])

    def row_copies(src, dst, sem, cuts):
        return [copy(src.at[pl.ds(a, b - a)], dst.at[pl.ds(a, b - a)], sem.at[i])
                for i, (a, b) in enumerate(zip(cuts, cuts[1:]))]

    def weight_terms(slot, a, n):
        halves = []
        for r in (a, a + n // 2):
            w = w_v[slot, pl.ds(r, n // 2), :]
            halves += [pltpu.bitcast(w << 16, f32), pltpu.bitcast(w & np.uint32(0xFFFF0000), f32)]
        return _rhs_terms(*halves)

    def q_weights(slot):
        return [t.astype(bf16) for t in weight_terms(slot, 0, M)]

    def kv_weights(slot):
        return [jnp.concatenate(t, axis=1).astype(bf16)
                for t in zip(weight_terms(slot, M, DC), weight_terms(slot, M + DC, DC))]

    def project_q(lhs, wts, a, b):
        for e, t in enumerate(_combine([_dot(_unpack(l), w) for l, w in zip(lhs, wts)])):
            q_v[e, a:b] = (t * QSCALE).astype(bf16)

    def project_kv(lhs, wts, a, b):
        for e, t in enumerate(_combine([_dot(_unpack(l), w) for l, w in zip(lhs, wts)])):
            k_v[e, a:b] = t[:, :D].astype(bf16)
            v_v[e, a:b] = t[:, D:].astype(bf16)

    def scores(qb, e, a, b):
        tri = (lax.broadcasted_iota(jnp.int32, (128, 128), 1)
               <= lax.broadcasted_iota(jnp.int32, (128, 128), 0))
        full = _dot_nt(qb, k_v[e, 0:a + 128])
        stairs = {t: _dot_nt(q_v[e, t:b], k_v[e, t:t + 128]) for t in range(a + 128, b, 128)}
        rows = []
        for r in range(a, b, 128):
            tiles = [full[r - a:r - a + 128, t:t + 128] for t in range(0, a + 128, 128)]
            tiles += [s[r - t:r - t + 128] for t, s in stairs.items() if t <= r]
            tiles[-1] = jnp.where(tri, tiles[-1], -1e30)
            rows.append(tiles)
        return rows

    def attend(rows, e, a, b):
        ps, sums = [], []
        for tiles in rows:
            top = jnp.max(_fold(jnp.maximum, tiles), axis=1, keepdims=True)
            ps.append([jnp.exp2(t - top) for t in tiles])
            sums.append(jnp.sum(_fold(jnp.add, ps[-1]), axis=1, keepdims=True))
        n0 = a // 128 + 1
        p = jnp.concatenate([jnp.concatenate(t[:n0], axis=1) for t in ps], axis=0)
        acc = _dot(p.astype(bf16), v_v[e, 0:a + 128])
        accs = [acc[i * 128:(i + 1) * 128] for i in range(len(ps))]
        for s in range(1, len(ps)):
            p = jnp.concatenate([t[n0 + s - 1] for t in ps[s:]], axis=0)
            acc = _dot(p.astype(bf16), v_v[e, a + s * 128:a + (s + 1) * 128])
            for i in range(s, len(ps)):
                accs[i] = accs[i] + acc[(i - s) * 128:(i - s + 1) * 128]
        out = []
        for acc, l in zip(accs, sums):
            r = pl.reciprocal(l, approx=True)
            out.append(acc * (r * (2.0 - l * r)))
        return out

    def head_pair(plan, j, slot):
        zero = (j >> 8).astype(u32)
        own = pl.ds(pl.multiple_of(j * 128, 128), 128)
        gate = jax.nn.sigmoid(jnp.sum(x_v[own].astype(f32) * row_v[5:6], axis=1, keepdims=True))
        gate = jnp.broadcast_to(gate, (128, 128))
        g_v[own] = gate
        bits = pltpu.bitcast(gate, u32)
        waiting = [(0 if slot is None else 1,
                    _fold(jnp.bitwise_or, [bits[i:i + 32] for i in range(0, 128, 32)]) & zero)]
        if slot is not None:
            wq, wkv = q_weights(slot), kv_weights(slot)
        step, pending, ctx = 0, {}, {}

        def paced(ref, a, b):
            lhs = [ref[i, a // 4:b // 4] for i in range(7)]
            for i in (2, 4, 6):
                if waiting and waiting[0][0] + 1 < step:
                    w, word = lhs[i], waiting.pop(0)[1]
                    ev, od = _unweave(w[:, :128], 8)
                    lhs[i] = jnp.concatenate([_weave(ev | word, od, 8), w[:, 128:]], axis=1)
            return lhs

        for kind, e, a, b in plan:
            if kind == "q":
                step += 1
                project_q(paced(xs_v, a, b), wq, a, b)
            elif kind == "kv":
                step += 1
                project_kv(paced(cs_v, a, b), wkv, a, b)
            elif kind == "qk":
                qb = q_v[e, a:b]
                if slot is None:
                    step += 1
                    if waiting and waiting[0][0] + 3 < step:
                        w = pltpu.bitcast(qb, u32)
                        qb = _unpack(jnp.concatenate([w[:32] | waiting.pop(0)[1], w[32:]], axis=0))
                pending[e, a] = scores(qb, e, a, b)
            else:
                for r, c in zip(range(a, b, 128), attend(pending.pop((e, a)), e, a, b)):
                    ctx[e, r] = c
                    if (1 - e, r) in ctx:
                        (a11, a21), (a12, a22) = _unweave(ctx[0, r]), _unweave(ctx[1, r])
                        terms = [_pack(t) for t in _lhs_terms(a11, a12, a21, a22)]
                        for i, t in enumerate(terms):
                            ctx_v[i, r // 4:(r + 128) // 4, own] = t
                        waiting.append((step, _fold(jnp.bitwise_or, terms) & zero))

    def input_terms(src, dst, a, b):
        ev, od = _unweave(src[a:b].astype(f32))
        n = ev.shape[1] // 2
        terms = [_pack(t) for t in _lhs_terms(ev[:, :n], ev[:, n:], od[:, :n], od[:, n:])]
        for i, t in enumerate(terms):
            dst[i, a // 4:b // 4] = t
        return terms

    c_in = row_copies(c_hbm, c_v, csem, C_ROWS)
    x_in = row_copies(x_hbm, x_v, xsem, X_ROWS)
    w_in = weight_copies(0, 0)
    small = [copy(a, b, ssem.at[i]) for i, (a, b) in enumerate(
        ((sk_hbm, sk_v), (sd_hbm, sd_v), (gw_hbm, gw_v), (fwd_hbm, fwd_v), (inv_hbm, inv_v)))]
    for cp in (c_in[0], w_in[1], w_in[2], c_in[1]):
        cp.start()
    w_in[1].wait()
    w_in[2].wait()
    for i, then in enumerate(([c_in[2]], [w_in[0], x_in[0], x_in[1]], x_in[2:])):
        c_in[i].wait()
        for cp in then:
            cp.start()
        if i == 0:
            wkv = kv_weights(0)
        for a in range(C_ROWS[i], C_ROWS[i + 1], 256):
            project_kv(input_terms(c_v, cs_v, a, a + 256), wkv, a, a + 256)
    w_in[0].wait()
    for i, cp in enumerate(x_in):
        cp.wait()
        if i == 0:
            wq = q_weights(0)
        if i == 1:
            for cp in small + weight_copies(1, 1):
                cp.start()
        for a in range(X_ROWS[i], X_ROWS[i + 1], 256):
            project_q(input_terms(x_v, xs_v, a, a + 256), wq, a, a + 256)
    for cp in small:
        cp.wait()
    row_v[0:4] = sk_v[...].astype(f32)
    row_v[4:5] = sd_v[...].astype(f32).reshape(1, M)
    row_v[5:6] = gw_v[...].astype(f32).reshape(1, M)

    loop_plan, last_plan = _plans()

    def pair_step(j, _):
        slot = (j + 1) % 2
        for cp in weight_copies(j + 1, slot):
            cp.wait()

        @pl.when(j + 2 < NP)
        def _():
            for cp in weight_copies(j + 2, 1 - slot):
                cp.start()

        head_pair(loop_plan, j, slot)
        return j + 1

    j_last = lax.fori_loop(0, NP - 1, pair_step, 0)
    for cp in block_copies(0, 0):
        cp.start()
    head_pair(last_plan, j_last, None)

    kp_v[0:8] = jnp.zeros((8, CB), f32)

    def spectra(slot, cs):
        fwd = fwd_v[...]
        taps = row_v[0:5, cs]
        prev = None
        for n in range(NB + H_LEAD):
            if n < NB:
                cur = _dot_nt(fwd, h_v[slot, :, n * T:(n + 1) * T])
                if prev is None:
                    H_v[n] = cur
                else:
                    (r0, r1), (i0, i1) = _unweave(cur[:T], 8), _unweave(cur[T:], 8)
                    (pr0, pr1), (pi0, pi1) = _unweave(prev[:T], 8), _unweave(prev[T:], 8)
                    H_v[n, :T] = _weave(r0 - pi0, r1 + pi1, 8)
                    H_v[n, T:] = _weave(i0 + pr0, i1 - pr1, 8)
                prev = cur
            if n >= H_LEAD:
                a = n - H_LEAD
                r = a * T
                kp_v[8 + r:8 + r + T] = bk_v[slot, r:r + T].astype(f32)
                ks = _fold(jnp.add, [kp_v[pl.ds(8 + r - t, T)] * taps[t:t + 1] for t in range(4)])
                u = ks * bv_v[slot, r:r + T].astype(f32)
                ud_v[r:r + T] = u * taps[4:5]
                U_v[a] = _dot(fwd, u.astype(bf16))

    def block_convolution(zero):
        words, done, total = {}, 0, (CB // 128) * (T // 16) * NB * (NB + 1) // 2

        def pace(w):
            tick = int(PACE_FROM + (PACE_TO - PACE_FROM) * done / total) // 16
            words[tick] = words[tick] | (w & zero) if tick in words else w & zero

        for c in range(0, CB, 128):
            ln = slice(c, c + 128)
            for f in range(0, T, 16):
                re, im = slice(f, f + 16), slice(T + f, T + f + 16)
                for a0 in range(0, NB, 2):
                    yr, yi, hs = [None, None], [None, None], {}
                    for s in range(a0 + 2):
                        ur, ui = U_v[s, re, ln], U_v[s, im, ln]
                        for o in range(2):
                            d = a0 + o - s
                            if d < 0:
                                continue
                            if d not in hs:
                                hs[d] = H_v[d, re, ln], H_v[d, im, ln]
                            hr, hi = hs[d]
                            pr, pi = hr * ur - hi * ui, hr * ui + hi * ur
                            yr[o] = pr if s == 0 else yr[o] + pr
                            yi[o] = pi if s == 0 else yi[o] + pi
                            done += 1
                        if s % 2 == 1 and s <= a0:
                            w = _fold(jnp.bitwise_or, [pltpu.bitcast(t, u32) for t in yr + yi])
                            pace(w[:8] | w[8:])
                    outs = []
                    for o in range(2):
                        r0, r1, i0, i1 = yr[o][:8], yr[o][8:], yi[o][:8], yi[o][8:]
                        for off, parts in ((0, (r0 + r1, i0 - i1)), (T, (r0 - r1, i0 + i1))):
                            outs.append(_pack(jnp.concatenate(parts, axis=0)))
                            Y_v[a0 + o, (off + f) // 2:(off + f) // 2 + 8, ln] = outs[-1]
                    pace(_fold(jnp.bitwise_or, outs))
        return words

    def channel_step(cb, _):
        slot = cb % 2
        cs = channels(cb)
        for cp in block_copies(cb, slot):
            cp.wait()
        spectra(slot, cs)

        @pl.when(cb + 1 < NCB)
        def _():
            for cp in block_copies(cb + 1, 1 - slot):
                cp.start()

        @pl.when(cb >= 2)
        def _():
            out_copy(cb - 2, slot, 0).wait()
            out_copy(cb - 2, slot, 1).wait()

        inv = inv_v[...]
        words = block_convolution((cb >> 8).astype(u32))
        wo = [jnp.concatenate([wo_v[slot, 2 * p + e, :, n:n + 128] for p in range(NP)], axis=0).astype(f32)
              for e in range(2) for n in (0, 128)]
        wo = [t.astype(bf16) for t in _rhs_terms(*wo)]
        att, ssm, tick = {}, {}, 0

        def mix(lo, hi):
            for r in range(lo, hi, T):
                g = g_v[r:r + T]
                g = jnp.concatenate([g, g], axis=1)
                o_v[slot, r:r + T] = (ssm[r] + g * (att[r] - ssm[r])).astype(bf16)

        for n, lo in enumerate(range(0, S, OM)):
            if n == INV_AT:
                for a in range(NB):
                    r = a * T
                    for par in range(2):
                        hf = slice(par * T // 2, (par + 1) * T // 2)
                        y = _dot(inv[hf], _unpack(Y_v[a, hf]))
                        for c in range(CB // 128):
                            y_v[c, pl.ds(r + par, T // 2, stride=2), :] = y[:, c * 128:(c + 1) * 128]
                    y = jnp.concatenate([y_v[c, r:r + T] for c in range(CB // 128)], axis=1)
                    ssm[r] = x_v[r:r + T, cs].astype(f32) * (y + ud_v[r:r + T])
                mix(0, lo)
                out_copy(cb, slot, 0).start()
            prods = []
            for i in range(7):
                cols = []
                for k in range(0, NP * D, 512):
                    rows = []
                    for r in range(lo // 4, (lo + OM) // 4, 8):
                        w = ctx_v[i, r:r + 8, k:k + 128]
                        rows.append(w | words[tick] if tick in words else w)
                        tick += 1
                    cols += [jnp.concatenate(rows, axis=0),
                             ctx_v[i, lo // 4:(lo + OM) // 4, k + 128:k + 512]]
                prods.append(_dot(_unpack(jnp.concatenate(cols, axis=1)), wo[i]))
            o = jnp.concatenate(_combine(prods), axis=1)
            for r in range(lo, lo + OM, T):
                att[r] = o[r - lo:r - lo + T]
            if n >= INV_AT:
                mix(lo, lo + OM)
        out_copy(cb, slot, 1).start()

    lax.fori_loop(0, NCB, channel_step, None)
    for cb in (NCB - 2, NCB - 1):
        out_copy(cb, cb % 2, 0).wait()
        out_copy(cb, cb % 2, 1).wait()


@jax.jit
def pallas_gated_mix__compressed_kv_cla__ssm_conv_h3__prompt_kernel(
    A_x: jax.Array,
    A_c_kv: jax.Array,
    A_w_q: jax.Array,
    A_w_uk: jax.Array,
    A_w_uv: jax.Array,
    A_w_o: jax.Array,
    B_q: jax.Array,
    B_k: jax.Array,
    B_v: jax.Array,
    B_shift_k: jax.Array,
    B_ssm_k: jax.Array,
    B_ssm_D: jax.Array,
    gate_w: jax.Array,
):
    del B_q
    vmem, sems = pltpu.VMEM, pltpu.SemaphoreType.DMA
    hbm = pl.BlockSpec(memory_space=pl.ANY)
    out = pl.pallas_call(
        _kernel,
        out_shape=jax.ShapeDtypeStruct((S, M), bf16),
        in_specs=[hbm] * 14,
        out_specs=hbm,
        scratch_shapes=[
            vmem((4, M), bf16), vmem((M,), bf16), vmem((M,), bf16),
            vmem((2 * T, T), bf16), vmem((T, T), bf16),
            vmem((S, M), bf16), vmem((S, DC), bf16),
            vmem((7, S // 4, M // 2), u32), vmem((7, S // 4, DC // 2), u32),
            vmem((2, M + 2 * DC, D), u32),
            vmem((2, S, D), bf16), vmem((2, S, D), bf16), vmem((2, S, D), bf16),
            vmem((7, S // 4, NP * D), u32),
            vmem((2, H, D, CB), bf16), vmem((2, S, CB), bf16), vmem((2, S, CB), bf16),
            vmem((2, CB, S), bf16),
            vmem((S, 128), f32), vmem((8, M), f32), vmem((S + 8, CB), f32), vmem((S, CB), f32),
            vmem((NB, 2 * T, CB), f32), vmem((NB, 2 * T, CB), f32), vmem((NB, T, CB), u32),
            vmem((CB // 128, S + 8, 128), f32), vmem((2, S, CB), bf16),
            sems((len(C_ROWS) - 1,)), sems((len(X_ROWS) - 1,)), sems((2, 3)), sems((2, 4)),
            sems((2, 2)), sems((5,)),
        ],
        compiler_params=pltpu.CompilerParams(vmem_limit_bytes=120 * 2**20, disable_bounds_checks=True),
    )(A_x.reshape(S, M), A_c_kv.reshape(S, DC), A_w_q, A_w_uk, A_w_uv, A_w_o,
      B_k.reshape(S, M), B_v.reshape(S, M), B_ssm_k, B_shift_k.T, B_ssm_D, gate_w,
      *_dft_matrices())
    return out.reshape(1, S, M)
```
